```python
import jax
import jax.numpy as jnp

def _softmax(x, axis=-1):
    return jax.nn.softmax(x, axis=axis)
def _gelu(x):
    return jax.nn.gelu(x, approximate=True)
def _silu(x):
    return jax.nn.silu(x)
def _sigmoid(x):
    return jax.nn.sigmoid(x)
def _layernorm(x, axis=-1, eps=1e-5):
    m = jnp.mean(x, axis=axis, keepdims=True)
    v = jnp.var(x, axis=axis, keepdims=True)
    return (x - m) / jnp.sqrt(v + eps)
def _scatter_add(tgt, idx, src, axis=0):
    return tgt.at[idx].add(src)
def _segment_sum(src, seg, n):
    return jax.ops.segment_sum(src, seg, n)
class _Rng:
    def __init__(self, key):
        self._k = key
    def _next(self):
        self._k, sub = jax.random.split(self._k)
        return sub
    def normal(self, shape):
        return jax.random.normal(self._next(), shape, dtype=jnp.bfloat16)
    def randint(self, lo, hi, shape):
        return jax.random.randint(self._next(), shape, lo, hi, dtype=jnp.int32)
    def uniform(self, shape, lo=0.0, hi=1.0):
        return jax.random.uniform(self._next(), shape, jnp.bfloat16, lo, hi)
    def permutation(self, n):
        return jax.random.permutation(self._next(), n)


kernel_name = 'interleave_layers__sliding_local_dilated__linear_kernel_hedgehog__prompt'

def setup_inputs():
    _rng = _Rng(jax.random.key(int.from_bytes(__import__("os").urandom(4), "little")))
    _w = (lambda a: (lambda t: t.astype(jnp.bfloat16) if jnp.issubdtype(t.dtype, jnp.floating) else t)(jnp.asarray(a)))
    def _A_setup():
        B, S, D = 1, 2048, 1024
        return {
            "x": _w((lambda *s: _rng.normal(s) * 0.05)(B, S, D)),
            "wqkv": _w((lambda *s: _rng.normal(s) * 0.05)(D, 3 * D)),
            "wo": _w((lambda *s: _rng.normal(s) * 0.05)(D, D)),
        }
    _A_in = _A_setup()

    def _B_setup():
        B, S, D, H = 1, 2048, 1024, 32
        Dh = D // H
        return {
            "x": _w((lambda *s: _rng.normal(s) * 0.05)(B, S, D)),
            "wqkv": _w((lambda *s: _rng.normal(s) * 0.05)(D, 3 * D)),
            "w_phi": _w((lambda *s: _rng.normal(s) * 0.05)(H, Dh, Dh) * (Dh ** -0.5)),
            "wo": _w((lambda *s: _rng.normal(s) * 0.05)(D, D)),
        }
    _B_in = _B_setup()

    return {
        "A_x": _A_in["x"],
        "A_wqkv": _A_in["wqkv"],
        "A_wo": _A_in["wo"],
        "B_x": _B_in["x"],
        "B_wqkv": _B_in["wqkv"],
        "B_w_phi": _B_in["w_phi"],
        "B_wo": _B_in["wo"],
    }

def reference(A_x, A_wqkv, A_wo, B_x, B_wqkv, B_w_phi, B_wo):
    def _A_ref(x, wqkv, wo):
        B, S, D = x.shape
        H = 32; Dh = D // H
        W, dil = 8, 2
        qkv = (lambda x, *d: x.transpose(*d))((x @ wqkv).reshape(B, S, 3, H, Dh), 2, 0, 3, 1, 4)
        q, k, v = qkv[0], qkv[1], qkv[2]
        scale = Dh ** -0.5
        pos = jnp.arange(S)
        off = jnp.arange(W) * dil
        idx = pos[:, None] - off[None, :]
        mask = idx >= 0
        idx_c = jnp.where(mask, idx, 0).reshape(-1)
        kg = k[:, :, idx_c, :].reshape(B, H, S, W, Dh)
        vg = v[:, :, idx_c, :].reshape(B, H, S, W, Dh)
        logits = jnp.einsum("bhsd,bhswd->bhsw", q, kg) * scale
        logits = jnp.where(mask[None, None, :, :], logits, -1e9)
        attn = _softmax(logits, axis=-1)
        o = jnp.einsum("bhsw,bhswd->bhsd", attn, vg)
        return (lambda x, *d: x.transpose(*d))(o, 0, 2, 1, 3).reshape(B, S, D) @ wo

    def _B_ref(x, wqkv, w_phi, wo):
        B, S, D = x.shape
        H = 32; Dh = D // H
        qkv = (lambda x, *d: x.transpose(*d))((x @ wqkv).reshape(B, S, 3, H, Dh), 2, 0, 3, 1, 4)
        q, k, v = qkv[0], qkv[1], qkv[2]
        pq = jnp.einsum("bhsd,hdf->bhsf", q, w_phi)
        pk = jnp.einsum("bhsd,hdf->bhsf", k, w_phi)
        phi_q = jnp.concatenate([_softmax(pq, axis=-1), _softmax(-pq, axis=-1)], axis=-1)
        phi_k = jnp.concatenate([_softmax(pk, axis=-1), _softmax(-pk, axis=-1)], axis=-1)
        kv = jnp.einsum("bhsf,bhsd->bhfd", phi_k, v)
        z  = jnp.einsum("bhsf->bhf", phi_k)
        num = jnp.einsum("bhqf,bhfd->bhqd", phi_q, kv)
        den = jnp.einsum("bhqf,bhf->bhq", phi_q, z)[..., None] + 1e-6
        o = num / den
        return (lambda x, *d: x.transpose(*d))(o, 0, 2, 1, 3).reshape(B, S, D) @ wo

    x = A_x
    x = x + _A_ref(_layernorm(x, axis=-1), A_wqkv, A_wo)
    x = x + _B_ref(_layernorm(x, axis=-1), B_wqkv, B_w_phi, B_wo)
    x = x + _A_ref(_layernorm(x, axis=-1), A_wqkv, A_wo)
    x = x + _B_ref(_layernorm(x, axis=-1), B_wqkv, B_w_phi, B_wo)
    return x
```

```python
import jax
import jax.numpy as jnp
from jax import lax
import jax.experimental.pallas as pl
import jax.experimental.pallas.tpu as pltpu

S, D, G, NC, CH = 2048, 1024, 8, 16, 512
LOG2E = 1.4426950408889634
F32, BF = jnp.float32, jnp.bfloat16
NT = (((1,), (1,)), ((), ()))


def _iota(shape, d):
    return lax.broadcasted_iota(jnp.int32, shape, d)


def _tree(f, xs):
    while len(xs) > 1:
        xs = [f(xs[i], xs[i + 1]) for i in range(0, len(xs), 2)]
    return xs[0]


def _body(x_hbm, aw_hbm, ao_hbm, bw_hbm, wp_ref, bo_hbm, out_ref,
          aw, ao, bw, bo, xt, ht, ot, wt, wot, buf0, buf1, stg, sems):
    cps = [pltpu.make_async_copy(s, d, sems.at[i]) for i, (s, d) in enumerate(
        [(x_hbm, out_ref), (aw_hbm, aw), (ao_hbm, ao), (bw_hbm, bw), (bo_hbm, bo)])]
    cps[0].start()
    cps[0].wait()
    for c in cps[1:]:
        c.start()

    def cols(i, n):
        return pl.ds(pl.multiple_of(i * n, n), n)

    def ln(sl):
        x = xt[:, sl]
        d = x - jnp.mean(x, axis=0, keepdims=True)
        v = jnp.mean(d * d, axis=0, keepdims=True)
        ht[:, sl] = (d * lax.rsqrt(v + 1e-5)).astype(BF)

    @pl.loop(0, 8)
    def _(i):
        v = out_ref[cols(i, 256), :].astype(F32)
        for r in range(8):
            vr = v[:, r * 128:(r + 1) * 128]
            stg[r, cols(i, 256), :] = vr

    @pl.loop(0, NC)
    def _(c):
        for r in range(8):
            xt[r * 128:(r + 1) * 128, cols(c, 128)] = stg[r, pl.ds(c, 128, stride=16), :].T
        ln(cols(c, 128))

    cps[1].wait()
    cps[2].wait()

    def proj(g, buf, c):
        sl = slice(c * CH, (c + 1) * CH)
        buf[0:384, sl] = jnp.dot(wt[g], ht[:, sl], preferred_element_type=F32)

    sub = _iota((8, 128), 0)
    lane0 = _iota((8, 128), 1) == 0

    def prep_a(g):
        for j in range(3):
            wt[g, j * 128:(j + 1) * 128, :] = aw[:, pl.ds(pl.multiple_of(j * D + g * 128, 128), 128)].T

    def merge(a, b, s):
        m = (sub & s) == 0
        return jnp.where(m, a + pltpu.roll(a, 8 - s, 0), b + pltpu.roll(b, s, 0))

    def att(g, buf, ch):
        if ch == 0:
            wot[g] = ao[cols(g, 128), :].T
            for h in range(8):
                rs = slice(128 + h * 32, 160 + h * 32)
                l0 = _iota((32, 128), 1) == 0
                first = pltpu.roll(buf[rs, 0:128], 1, 1)
                for c in range(2, 16):
                    r = pltpu.roll(buf[rs, c * 128:(c + 1) * 128], 1, 1)
                    buf[rs, (14 + c) * 128:(15 + c) * 128] = jnp.where(l0, first, r)
        h = ch
        for c in range(NC):
            q = buf[h * 32:h * 32 + 32, c * 128:(c + 1) * 128]
            ls = []
            for j in range(8):
                e = (c - 2 * j) % 30
                p = q * buf[128 + h * 32:160 + h * 32, e * 128:(e + 1) * 128]
                ls.append((p[0:8] + p[8:16]) + (p[16:24] + p[24:32]))
            ls = [merge(ls[i], ls[i + 4], 4) for i in range(4)]
            ls = [merge(ls[i], ls[i + 2], 2) for i in range(2)]
            lg = merge(ls[0], ls[1], 1) * (32 ** -0.5 * LOG2E)
            if c < 14:
                lg = jnp.where(lane0 & (2 * sub > c), -1e9 * LOG2E, lg)
            ex = jnp.exp2(lg - jnp.max(lg, axis=0, keepdims=True))
            pr = ex / jnp.sum(ex, axis=0, keepdims=True)
            os_ = []
            for j in range(8):
                e = c - 2 * j
                e = e if e >= 0 else e + 30
                os_.append(pr[j:j + 1, :] * buf[256 + h * 32:288 + h * 32, e * 128:(e + 1) * 128])
            ot[pl.ds(pl.multiple_of(g * 128 + h * 32, 32), 32),
               c * 128:(c + 1) * 128] = _tree(jnp.add, os_).astype(BF)

    def prep_b(g):
        r, cc = _iota((128, 128), 0), _iota((128, 128), 1)
        sel = (_iota((128, 32), 0) // 4 == _iota((128, 32), 1)).astype(BF)
        t = lax.dot_general(sel, wp_ref[cols(g, 128), :], NT, preferred_element_type=F32)
        m = jnp.where(r % 4 == cc // 32, t, 0.0).astype(BF)
        for j in range(2):
            w = bw[:, pl.ds(pl.multiple_of(j * D + g * 128, 128), 128)]
            wt[g, j * 128:(j + 1) * 128, :] = (
                lax.dot_general(m, w, NT, preferred_element_type=F32) * LOG2E).astype(BF)
        wt[g, 256:384, :] = bw[:, pl.ds(pl.multiple_of(2 * D + g * 128, 128), 128)].T

    def phi(buf, r0, c):
        a, b = [], []
        for k in range(c * 4, c * 4 + 4):
            p = buf[r0:r0 + 128, k * 128:(k + 1) * 128].reshape(16, 8, 128)
            res = []
            for red, sg in ((jnp.maximum, 1), (jnp.minimum, -1)):
                m = _tree(red, [p[i] for i in range(16)])
                m = red(m, pltpu.roll(m, 4, 0))
                e = jnp.exp2(p - m[None] if sg > 0 else m[None] - p)
                s = _tree(jnp.add, [e[i] for i in range(16)])
                s = 1.0 / (s + pltpu.roll(s, 4, 0))
                res.append((e * s[None]).reshape(128, 128).astype(BF))
            a.append(jnp.concatenate(res, axis=0))
        return jnp.concatenate(a, axis=1)

    def lin(g, buf, ch, kv):
        if ch == 0:
            wot[g] = bo[cols(g, 128), :].T
        if ch < 2:
            for c in (2 * ch, 2 * ch + 1):
                v = jnp.concatenate([buf[256:384, c * CH:(c + 1) * CH], jnp.ones((32, CH), F32)], axis=0)
                t = lax.dot_general(v.astype(BF), phi(buf, 128, c), NT, preferred_element_type=F32)
                kv = t if kv is None else kv + t
            if ch == 1:
                r, cc = _iota((160, 256), 0), _iota((160, 256), 1)
                hd = jnp.where(r < 128, r // 32, (r - 128) // 8)
                kv = jnp.where(hd == cc % 4, kv, 0.0).astype(BF)
            return kv
        for c in (2 * ch - 4, 2 * ch - 3):
            t = jnp.dot(kv, phi(buf, 0, c), preferred_element_type=F32)
            inv = 1.0 / (t[128:160].reshape(4, 1, 8, CH) + 1e-6)
            o = t[0:128].reshape(4, 4, 8, CH) * inv
            ot[cols(g, 128), c * CH:(c + 1) * CH] = o.reshape(128, CH).astype(BF)
        return kv

    def groups(prep, post):
        prep(0)
        prep(1)
        for c in range(4):
            proj(0, buf0, c)

        def step(g, cur, nxt, last=False):
            st = None
            for c in range(4):
                if not last:
                    proj(g + 1, nxt, c)
                st = post(g, cur, c) if post is att else post(g, cur, c, st)
                if c == 2 and not last:
                    prep(jnp.minimum(g + 2, G - 1)) if post is att else prep((g + 2) % G)

        @pl.loop(0, 3)
        def _(i):
            step(2 * i, buf0, buf1)
            step(2 * i + 1, buf1, buf0)
        step(jnp.int32(6), buf0, buf1)
        step(jnp.int32(7), buf1, buf0, last=True)

        def mm(i):
            w = jnp.concatenate([wot[g] for g in range(G)], axis=1)
            xt[:, cols(i, 256)] += jnp.dot(w, ot[:, cols(i, 256)], preferred_element_type=F32)
        mm(0)

        @pl.loop(1, 8)
        def _(i):
            ln(cols(i - 1, 256))
            mm(i)
        ln(cols(7, 256))

    @pl.loop(0, 2)
    def _(it):
        groups(prep_a, att)

        @pl.when(it == 0)
        def _():
            cps[3].wait()
            cps[4].wait()
        groups(prep_b, lin)

    @pl.loop(0, NC)
    def _(c):
        for r in range(8):
            stg[r, pl.ds(c, 128, stride=16), :] = xt[r * 128:(r + 1) * 128, cols(c, 128)].T

    @pl.loop(0, 8)
    def _(i):
        for r in range(8):
            out_ref[cols(i, 256), r * 128:(r + 1) * 128] = stg[r, cols(i, 256), :].astype(BF)


@jax.jit
def pallas_interleave_layers__sliding_local_dilated__linear_kernel_hedgehog__prompt_kernel(
        A_x, A_wqkv, A_wo, B_x, B_wqkv, B_w_phi, B_wo):
    hbm = pl.BlockSpec(memory_space=pl.ANY)
    vm = pl.BlockSpec(memory_space=pltpu.VMEM)
    V = pltpu.VMEM
    out = pl.pallas_call(
        _body,
        in_specs=[hbm, hbm, hbm, hbm, vm, hbm],
        out_specs=vm,
        out_shape=jax.ShapeDtypeStruct((S, D), BF),
        scratch_shapes=[V((D, 3 * D), BF), V((D, D), BF), V((D, 3 * D), BF), V((D, D), BF),
                        V((D, S), F32), V((D, S), BF), V((D, S), BF), V((G, 384, D), BF),
                        V((G, D, 128), BF), V((384, 30 * 128), F32), V((384, 30 * 128), F32), V((8, S, 128), F32),
                        pltpu.SemaphoreType.DMA((5,))],
        compiler_params=pltpu.CompilerParams(vmem_limit_bytes=110 * 2**20),
    )(A_x.reshape(S, D), A_wqkv, A_wo, B_wqkv, B_w_phi.reshape(D, 32), B_wo)
    return out.reshape(1, S, D)
```

```python
import jax
import jax.numpy as jnp
from jax import lax
import jax.experimental.pallas as pl
import jax.experimental.pallas.tpu as pltpu

S, D, G, NC, CH = 2048, 1024, 8, 16, 512
LOG2E = 1.4426950408889634
F32, BF = jnp.float32, jnp.bfloat16
NT = (((1,), (1,)), ((), ()))


def _iota(shape, d):
    return lax.broadcasted_iota(jnp.int32, shape, d)


def _tree(f, xs):
    while len(xs) > 1:
        xs = [f(xs[i], xs[i + 1]) for i in range(0, len(xs), 2)]
    return xs[0]


def _body(x_hbm, aw_hbm, ao_hbm, bw_hbm, wp_ref, bo_hbm, out_ref,
          aw, ao, bw, bo, xt, ht, ot, wt, wot, buf0, buf1, stg, sems):
    xin = [pltpu.make_async_copy(x_hbm.at[:, r * 128:(r + 1) * 128], stg.at[r], sems.at[5 + r]) for r in range(8)]
    xout = [pltpu.make_async_copy(stg.at[r], out_ref.at[:, r * 128:(r + 1) * 128], sems.at[5 + r]) for r in range(8)]
    cps = [None] + [pltpu.make_async_copy(s, d, sems.at[i]) for i, (s, d) in enumerate(
        [(aw_hbm, aw), (ao_hbm, ao), (bw_hbm, bw), (bo_hbm, bo)])]
    for c in xin:
        c.start()
    cps[1].start()
    for c in xin:
        c.wait()
    st32 = stg.bitcast(jnp.int32)

    def cols(i, n):
        return pl.ds(i * n, n) if isinstance(i, int) else pl.ds(pl.multiple_of(i * n, n), n)

    def ln(sl):
        x = xt[:, sl]
        d = x - jnp.mean(x, axis=0, keepdims=True)
        v = jnp.mean(d * d, axis=0, keepdims=True)
        ht[:, sl] = (d * lax.rsqrt(v + 1e-5)).astype(BF)

    for m in range(8):
        for r in range(8):
            w = st32[r, pl.ds(m, 128, stride=8), :].T
            xt[r * 128:(r + 1) * 128, cols(2 * m, 128)] = pltpu.bitcast(w << 16, F32)
            xt[r * 128:(r + 1) * 128, cols(2 * m + 1, 128)] = pltpu.bitcast(w & -65536, F32)
        ln(cols(m, 256))

    cps[1].wait()
    for c in cps[2:]:
        c.start()

    def emit(m):
        for r in range(8):
            v = pltpu.bitcast(xt[r * 128:(r + 1) * 128, cols(m, 256)].astype(BF).astype(F32), jnp.int32)
            w = v[:, 128:] | lax.shift_right_logical(v[:, :128], 16)
            st32[r, pl.ds(m, 128, stride=8), :] = w.T

    def proj(g, buf, c):
        if c % 2: return
        sl = slice(c * CH, (c + 2) * CH)
        buf[0:384, sl] = jnp.dot(wt[g], ht[:, sl], preferred_element_type=F32)

    sub = _iota((8, 128), 0)
    lane0 = _iota((8, 128), 1) == 0

    def prep_a(g):
        for j in range(3):
            wt[g, j * 128:(j + 1) * 128, :] = aw[:, pl.ds(pl.multiple_of(j * D + g * 128, 128), 128)].T

    def merge(a, b, s):
        m = (sub & s) == 0
        return jnp.where(m, a + pltpu.roll(a, 8 - s, 0), b + pltpu.roll(b, s, 0))

    def att(g, buf, ch):
        if ch == 0:
            wot[g] = ao[cols(g, 128), :].T
            for h in range(8):
                rs = slice(128 + h * 32, 160 + h * 32)
                l0 = _iota((32, 128), 1) == 0
                first = pltpu.roll(buf[rs, 0:128], 1, 1)
                for c in range(2, 16):
                    r = pltpu.roll(buf[rs, c * 128:(c + 1) * 128], 1, 1)
                    buf[rs, (14 + c) * 128:(15 + c) * 128] = jnp.where(l0, first, r)
        h = ch
        for c in range(NC):
            q = buf[h * 32:h * 32 + 32, c * 128:(c + 1) * 128]
            ls = []
            for j in range(8):
                e = (c - 2 * j) % 30
                p = q * buf[128 + h * 32:160 + h * 32, e * 128:(e + 1) * 128]
                ls.append((p[0:8] + p[8:16]) + (p[16:24] + p[24:32]))
            ls = [merge(ls[i], ls[i + 4], 4) for i in range(4)]
            ls = [merge(ls[i], ls[i + 2], 2) for i in range(2)]
            lg = merge(ls[0], ls[1], 1) * (32 ** -0.5 * LOG2E)
            if c < 14:
                lg = jnp.where(lane0 & (2 * sub > c), -1e9 * LOG2E, lg)
            ex = jnp.exp2(lg - jnp.max(lg, axis=0, keepdims=True))
            pr = ex / jnp.sum(ex, axis=0, keepdims=True)
            os_ = []
            for j in range(8):
                e = c - 2 * j
                e = e if e >= 0 else e + 30
                os_.append(pr[j:j + 1, :] * buf[256 + h * 32:288 + h * 32, e * 128:(e + 1) * 128])
            ot[pl.ds(pl.multiple_of(g * 128 + h * 32, 32), 32),
               c * 128:(c + 1) * 128] = _tree(jnp.add, os_).astype(BF)

    def prep_b(g):
        r, cc = _iota((128, 128), 0), _iota((128, 128), 1)
        sel = (_iota((128, 32), 0) // 4 == _iota((128, 32), 1)).astype(BF)
        t = lax.dot_general(sel, wp_ref[cols(g, 128), :], NT, preferred_element_type=F32)
        m = jnp.where(r % 4 == cc // 32, t, 0.0).astype(BF)
        for j in range(2):
            w = bw[:, pl.ds(pl.multiple_of(j * D + g * 128, 128), 128)]
            wt[g, j * 128:(j + 1) * 128, :] = (
                lax.dot_general(m, w, NT, preferred_element_type=F32) * LOG2E).astype(BF)
        wt[g, 256:384, :] = bw[:, pl.ds(pl.multiple_of(2 * D + g * 128, 128), 128)].T

    def phi(buf, r0, c):
        a, z = [], []
        for k in range(c * 4, c * 4 + 4):
            p = buf[r0:r0 + 128, k * 128:(k + 1) * 128].reshape(16, 8, 128)
            res = []
            for red, sg in ((jnp.maximum, 1), (jnp.minimum, -1)):
                m = _tree(red, [p[i] for i in range(16)])
                m = red(m, pltpu.roll(m, 4, 0))
                e = jnp.exp2(p - m[None] if sg > 0 else m[None] - p)
                s = _tree(jnp.add, [e[i] for i in range(16)])
                s = 1.0 / (s + pltpu.roll(s, 4, 0))
                res.append((e * s[None]).reshape(128, 128))
            z.append(jnp.concatenate(res, axis=0))
            a.append(z[-1].astype(BF))
        return jnp.concatenate(a, axis=1), _tree(jnp.add, z)

    def lin(g, buf, ch, kv):
        if ch == 0:
            wot[g] = bo[cols(g, 128), :].T
        if ch < 2:
            for c in (2 * ch, 2 * ch + 1):
                v = buf[256:384, c * CH:(c + 1) * CH].astype(BF)
                p, z = phi(buf, 128, c)
                t = lax.dot_general(p, v, NT, preferred_element_type=F32)
                kv = (t, z) if kv is None else (kv[0] + t, kv[1] + z)
            if ch == 1:
                z = jnp.broadcast_to(jnp.sum(kv[1].T, axis=0, keepdims=True), (32, 256))
                kv = jnp.concatenate([kv[0].T, z], axis=0)
                r, cc = _iota((160, 256), 0), _iota((160, 256), 1)
                hd = jnp.where(r < 128, r // 32, (r - 128) // 8)
                kv = jnp.where(hd == cc % 4, kv, 0.0).astype(BF)
            return kv
        for c in (2 * ch - 4, 2 * ch - 3):
            t = jnp.dot(kv, phi(buf, 0, c)[0], preferred_element_type=F32)
            inv = 1.0 / (t[128:160].reshape(4, 1, 8, CH) + 1e-6)
            o = t[0:128].reshape(4, 4, 8, CH) * inv
            ot[cols(g, 128), c * CH:(c + 1) * CH] = o.reshape(128, CH).astype(BF)
        return kv

    def groups(prep, post, it):
        prep(0)
        prep(1)
        for c in range(4):
            proj(0, buf0, c)
        if post is att:
            @pl.when(it == 0)
            def _():
                cps[2].wait()

        def step(g, cur, nxt, last=False):
            st = None
            for c in range(4):
                if not last:
                    proj(g + 1, nxt, c)
                st = post(g, cur, c) if post is att else post(g, cur, c, st)
                if c == 2 and not last:
                    prep(jnp.minimum(g + 2, G - 1)) if post is att else prep((g + 2) % G)

        @pl.loop(0, 3)
        def _(i):
            step(2 * i, buf0, buf1)
            step(2 * i + 1, buf1, buf0)
        step(jnp.int32(6), buf0, buf1)
        step(jnp.int32(7), buf1, buf0, last=True)

        def mm(i):
            w = jnp.concatenate([wot[g] for g in range(G)], axis=1)
            xt[:, cols(i, 256)] += jnp.dot(w, ot[:, cols(i, 256)], preferred_element_type=F32)
        mm(0)

        def rest(fin):
            @pl.loop(1, 8)
            def _(i):
                fin(i - 1)
                mm(i)
        if post is att:
            rest(lambda i: ln(cols(i, 256)))
        else:
            pl.when(it == 0)(lambda: rest(lambda i: ln(cols(i, 256))))
            pl.when(it == 1)(lambda: [(emit(i - 1), mm(i))[0] for i in range(1, 8)] and None)
        if post is att:
            ln(cols(7, 256))
        else:
            pl.when(it == 0)(lambda: ln(cols(7, 256)))

    @pl.loop(0, 2)
    def _(it):
        groups(prep_a, att, it)

        @pl.when(it == 0)
        def _():
            cps[3].wait()
            cps[4].wait()
        groups(prep_b, lin, it)

    emit(7)
    for c in xout:
        c.start()
    for c in xout:
        c.wait()


@jax.jit
def pallas_interleave_layers__sliding_local_dilated__linear_kernel_hedgehog__prompt_kernel(
        A_x, A_wqkv, A_wo, B_x, B_wqkv, B_w_phi, B_wo):
    hbm = pl.BlockSpec(memory_space=pl.ANY)
    vm = pl.BlockSpec(memory_space=pltpu.VMEM)
    V = pltpu.VMEM
    out = pl.pallas_call(
        _body,
        in_specs=[hbm, hbm, hbm, hbm, vm, hbm],
        out_specs=hbm,
        out_shape=jax.ShapeDtypeStruct((S, D), BF),
        scratch_shapes=[V((D, 3 * D), BF), V((D, D), BF), V((D, 3 * D), BF), V((D, D), BF),
                        V((D, S), F32), V((D, S), BF), V((D, S), BF), V((G, 384, D), BF),
                        V((G, D, 128), BF), V((384, 30 * 128), F32), V((384, 30 * 128), F32), V((8, S, 128), BF),
                        pltpu.SemaphoreType.DMA((13,))],
        compiler_params=pltpu.CompilerParams(vmem_limit_bytes=110 * 2**20),
    )(A_x.reshape(S, D), A_wqkv, A_wo, B_wqkv, B_w_phi.reshape(D, 32), B_wo)
    return out.reshape(1, S, D)
```
